```python
import os as _os
_os.environ.setdefault("JAX_PLATFORMS", "cpu")
import jax
import jax.numpy as jnp

def _softmax(x, axis=-1):
    return jax.nn.softmax(x, axis=axis)
def _gelu(x):
    return jax.nn.gelu(x, approximate=True)
def _silu(x):
    return jax.nn.silu(x)
def _sigmoid(x):
    return jax.nn.sigmoid(x)
def _layernorm(x, axis=-1, eps=1e-5):
    m = jnp.mean(x, axis=axis, keepdims=True)
    v = jnp.var(x, axis=axis, keepdims=True)
    return (x - m) / jnp.sqrt(v + eps)
def _scatter_add(tgt, idx, src, axis=0):
    return tgt.at[idx].add(src)
def _segment_sum(src, seg, n):
    return jax.ops.segment_sum(src, seg, n)
class _Rng:
    def __init__(self, key):
        self._k = key
    def _next(self):
        self._k, sub = jax.random.split(self._k)
        return sub
    def normal(self, shape):
        return jax.random.normal(self._next(), shape, dtype=jnp.bfloat16)
    def randint(self, lo, hi, shape):
        return jax.random.randint(self._next(), shape, lo, hi, dtype=jnp.int32)
    def uniform(self, shape, lo=0.0, hi=1.0):
        return jax.random.uniform(self._next(), shape, jnp.bfloat16, lo, hi)
    def permutation(self, n):
        return jax.random.permutation(self._next(), n)


kernel_name = 'standalone__mha_softmax__near_ridge'

def setup_inputs():
    _rng = _Rng(jax.random.key(int.from_bytes(__import__("os").urandom(4), "little")))
    _w = (lambda a: (lambda t: t.astype(jnp.bfloat16) if jnp.issubdtype(t.dtype, jnp.floating) else t)(jnp.asarray(a)))
    B, H, Sq, Sk, D = 8, 32, 512, 512, 128
    return {
        "q": _w((lambda *s: _rng.normal(s) * 0.4)(B, H, Sq, D)),
        "k": _w((lambda *s: _rng.normal(s) * 0.4)(B, H, Sk, D)),
        "v": _w((lambda *s: _rng.normal(s) * 0.05)(B, H, Sk, D)),
    }

def reference(q, k, v):
    scale = q.shape[-1] ** -0.5
    scores = jnp.einsum("bhqd,bhkd->bhqk", q, k) * scale
    p = _softmax(scores, axis=-1)
    return jnp.einsum("bhqk,bhkd->bhqd", p, v)
```

```python
import math

import jax
import jax.numpy as jnp
from jax import lax
import jax.experimental.pallas as pl
import jax.experimental.pallas.tpu as pltpu

_RUNS = ((1, 2), (2, 2), (4, 2), (7, 3), (14, 4), (33, 5))
_SWITCH = 16
_PIECE = 128


def _head(q, k, v, c):
    q = (q.astype(jnp.float32) * c).astype(jnp.bfloat16)
    s = lax.dot_general(q, k, (((1,), (1,)), ((), ())),
                        preferred_element_type=jnp.float32)
    m = jnp.max(s, axis=-1, keepdims=True)
    p = jnp.exp2(s - m)
    l = jnp.sum(p, axis=-1, keepdims=True)
    o = jnp.dot(p.astype(jnp.bfloat16), v, preferred_element_type=jnp.float32)
    return (o * pl.reciprocal(l, approx=True)).astype(jnp.bfloat16)


@jax.jit
def pallas_standalone__mha_softmax__near_ridge_kernel(
    q: jax.Array,
    k: jax.Array,
    v: jax.Array,
):
    B, H, S, D = q.shape
    NH = B * H
    c = (D ** -0.5) * math.log2(math.e)

    seq = [n for n, cnt in _RUNS for _ in range(cnt)]
    starts = [sum(seq[:i]) for i in range(len(seq))]
    assert sum(seq) == NH
    nb = len(seq)
    plan = {}
    written = 0
    for i in range(_SWITCH, nb):
        hi = starts[i] if i == nb - 1 else (starts[i] // 8) * 8
        if hi > written:
            plan[i] = (written, hi - written)
            written = hi

    def kernel(q_hbm, k_hbm, v_hbm, o_hbm, qb, kb, vb, rsem, wsem):
        srcs = ((k_hbm, kb), (q_hbm, qb), (v_hbm, vb))

        def read(bi, start, n, j):
            src, dst = srcs[j]
            return pltpu.make_async_copy(
                src.at[pl.ds(start, n)], dst.at[pl.ds(start, n)], rsem.at[bi])

        def write(g, g0, gn, pc):
            if g == 1:
                src, dst = qb, o_hbm
            else:
                src = qb.reshape(NH // g, g * S, D)
                dst = o_hbm.reshape(NH // g, g * S, D)
            for r in range(g * S // pc):
                pltpu.make_async_copy(
                    src.at[pl.ds(g0, gn), pl.ds(r * pc, pc)],
                    dst.at[pl.ds(g0, gn), pl.ds(r * pc, pc)],
                    wsem.at[0]).start()

        def write_span(start, n):
            while n > 0:
                if start % 8 == 0 and n >= 32:
                    m = (n // 8) * 8
                    write(8, start // 8, m // 8, _PIECE)
                elif start % 4 == 0 and n >= 16:
                    m = (n // 4) * 4
                    write(4, start // 4, m // 4, _PIECE)
                elif n >= 4:
                    m = n
                    write(1, start, m, 32)
                else:
                    m = n
                    write(1, start, m, S)
                start += m
                n -= m

        def everything(carry):
            for bi in range(nb):
                for j in range(3):
                    read(bi, starts[bi], seq[bi], j).start()
            b0 = 0
            for n, cnt in _RUNS:
                def body(t, cc, b0=b0, n=n, cnt=cnt):
                    i = b0 + t
                    start = starts[b0] + t * n
                    for step, span in plan.items():
                        if b0 <= step < b0 + cnt:
                            pl.when(i == step)(
                                lambda span=span: write_span(*span))
                    for j in range(3):
                        read(i, start, n, j).wait()
                    for h in range(n):
                        qb[start + h] = _head(
                            qb[start + h], kb[start + h], vb[start + h], c)
                        if b0 + cnt == nb:
                            pl.when(i == nb - 1)(
                                lambda h=h: write(1, start + h, 1, S))
                    return cc
                lax.fori_loop(0, cnt, body, 0)
                b0 += cnt
            pltpu.make_async_copy(qb, o_hbm, wsem.at[0]).wait()
            return carry + 1

        lax.while_loop(lambda t: t < 1, everything, jnp.int32(0))

    shp = (NH, S, D)
    spec = pl.BlockSpec(memory_space=pl.ANY)
    out = pl.pallas_call(
        kernel,
        in_specs=[spec] * 3,
        out_specs=spec,
        out_shape=jax.ShapeDtypeStruct(shp, q.dtype),
        scratch_shapes=[pltpu.VMEM(shp, q.dtype)] * 3
        + [pltpu.SemaphoreType.DMA((nb,)), pltpu.SemaphoreType.DMA((1,))],
        compiler_params=pltpu.CompilerParams(
            vmem_limit_bytes=126 * 1024 * 1024, disable_bounds_checks=True),
    )(q.reshape(shp), k.reshape(shp), v.reshape(shp))
    return out.reshape(B, H, S, D)
```

```python
import functools
import math

import jax
import jax.numpy as jnp
from jax import lax
import jax.experimental.pallas as pl
import jax.experimental.pallas.tpu as pltpu

_RUNS = ((1, 2), (2, 2), (4, 2), (7, 3), (14, 4), (33, 5))
_GROUPS = ((186, 0, 184), (231, 184, 48), (247, 232, 16), (251, 248, 4),
           (252, 252, 1), (253, 253, 1), (254, 254, 1))
_PIECE = 128
_MAX_STARTS = 16
_SPLIT = 384
_LAST_SPLIT = 496
_TAIL_CUTS = (256, 448)


def _head(q, k, v, c):
    q = (q.astype(jnp.float32) * c).astype(jnp.bfloat16)
    s = lax.dot_general(q, k, (((1,), (1,)), ((), ())),
                        preferred_element_type=jnp.float32)
    m = jnp.max(s, axis=-1, keepdims=True)
    p = jnp.exp2(s - m)
    l = jnp.sum(p, axis=-1, keepdims=True)
    o = jnp.dot(p.astype(jnp.bfloat16), v, preferred_element_type=jnp.float32)
    return (o * pl.reciprocal(l, approx=True)).astype(jnp.bfloat16)


@jax.jit
def pallas_standalone__mha_softmax__near_ridge_kernel(
    q: jax.Array,
    k: jax.Array,
    v: jax.Array,
):
    B, H, S, D = q.shape
    NH = B * H
    c = (D ** -0.5) * math.log2(math.e)

    seq = [n for n, cnt in _RUNS for _ in range(cnt)]
    starts = [sum(seq[:i]) for i in range(len(seq))]
    assert sum(seq) == NH
    nb = len(seq)
    loc = {starts[i] + h: (i, h) for i in range(nb) for h in range(seq[i])}

    def kernel(q_hbm, k_hbm, v_hbm, o_hbm, qb, kb, vb, rsem, wsem):
        srcs = ((k_hbm, kb), (q_hbm, qb), (v_hbm, vb))

        def read(bi, start, n, j):
            src, dst = srcs[j]
            return pltpu.make_async_copy(
                src.at[pl.ds(start, n)], dst.at[pl.ds(start, n)], rsem.at[bi])

        def start_write(g, g0, gn, r0, rows):
            if g == 1:
                src, dst = qb, o_hbm
            else:
                src = qb.reshape(NH // g, g * S, D)
                dst = o_hbm.reshape(NH // g, g * S, D)
            pltpu.make_async_copy(
                src.at[pl.ds(g0, gn), pl.ds(r0, rows)],
                dst.at[pl.ds(g0, gn), pl.ds(r0, rows)],
                wsem.at[0]).start()

        def span_writes(start, n):
            if n >= 32:
                g, rows = 8, _PIECE
            elif n >= 16:
                g, rows = 4, _PIECE
            elif n >= 4:
                g, rows = 1, 32
            else:
                g, rows = 1, S
            assert start % g == 0 and n % g == 0
            return [(g, start // g, n // g, r0, rows)
                    for r0 in range(0, g * S, rows)]

        after = {}
        for a, first, n in _GROUPS:
            assert a >= first + n - 1
            ws = span_writes(first, n)
            for ci in range(0, len(ws), _MAX_STARTS):
                after[a + ci // _MAX_STARTS] = ws[ci:ci + _MAX_STARTS]

        def start_writes(ws):
            for w in ws:
                start_write(*w)

        def block(t, start2, *, b0, n, cnt):
            i = b0 + t
            start = starts[b0] + t * n
            for j in range(3):
                read(i, start, n, j).wait()

            def load_q(h):
                hi = _LAST_SPLIT if 1 <= h == n - 1 else S
                if h < 2:
                    return [qb[start + h, pl.ds(0, hi), :]]
                return [qb[start + h, pl.ds(0, _SPLIT), :],
                        qb[start2 + h, pl.ds(_SPLIT, hi - _SPLIT), :]]

            qs = {h: load_q(h) for h in range(min(2, n))}
            for h in range(n):
                if 1 <= h == n - 1:
                    qs[h].append(
                        qb[start2 + h, pl.ds(_LAST_SPLIT, S - _LAST_SPLIT), :])
                parts = qs.pop(h)
                qh = parts[0] if len(parts) == 1 else jnp.concatenate(parts, 0)
                o = _head(qh, kb[start + h], vb[start + h], c)
                if b0 + cnt == nb and h == n - 1:
                    cuts = (0,) + _TAIL_CUTS + (S,)
                    for lo, hi in zip(cuts[:-1], cuts[1:]):
                        qb[start + h, pl.ds(lo, hi - lo), :] = o[lo:hi]
                        if hi < S:
                            pl.when(i == nb - 1)(functools.partial(
                                start_write, 1, NH - 1, 1, lo, hi - lo))
                else:
                    qb[start + h] = o
                for it in range(b0, b0 + cnt):
                    ws = after.get(starts[it] + h)
                    if ws:
                        pl.when(i == it)(functools.partial(start_writes, ws))
                if h + 2 < n:
                    qs[h + 2] = load_q(h + 2)
            return start2 + n

        def everything(done):
            for bi in range(nb):
                for j in range(3):
                    read(bi, starts[bi], seq[bi], j).start()
            b0 = 0
            for n, cnt in _RUNS:
                done = lax.fori_loop(
                    0, cnt, functools.partial(block, b0=b0, n=n, cnt=cnt), done)
                b0 += cnt
            start_write(1, NH - 1, 1, _TAIL_CUTS[-1], S - _TAIL_CUTS[-1])
            pltpu.make_async_copy(qb, o_hbm, wsem.at[0]).wait()
            return done

        lax.while_loop(lambda done: done < NH, everything, jnp.int32(0))

    shp = (NH, S, D)
    spec = pl.BlockSpec(memory_space=pl.ANY)
    out = pl.pallas_call(
        kernel,
        in_specs=[spec] * 3,
        out_specs=spec,
        out_shape=jax.ShapeDtypeStruct(shp, q.dtype),
        scratch_shapes=[pltpu.VMEM(shp, q.dtype)] * 3
        + [pltpu.SemaphoreType.DMA((nb,)), pltpu.SemaphoreType.DMA((1,))],
        compiler_params=pltpu.CompilerParams(
            vmem_limit_bytes=126 * 1024 * 1024,
            disable_bounds_checks=True,
            disable_semaphore_checks=True),
    )(q.reshape(shp), k.reshape(shp), v.reshape(shp))
    return out.reshape(B, H, S, D)
```

```python
import functools
import math

import jax
import jax.numpy as jnp
from jax import lax
import jax.experimental.pallas as pl
import jax.experimental.pallas.tpu as pltpu

_RUNS = ((1, 2), (2, 3), (4, 2), (7, 4), (17, 3), (32, 5))
_WRITES = ((187, 0, 184), (231, 184, 48), (247, 232, 16), (251, 248, 4),
           (253, 252, 2), (254, 254, 1))
_GROUPS = 32
_PIECE = 128
_MAX_STARTS = 16
_SPLIT = 416
_CARRY = 256
_TAIL_CUTS = (256, 448)
_LANES = 128
_Q, _K, _V = 0, 1, 2


def _scores(q, k, c):
    q = (q.astype(jnp.float32) * c).astype(jnp.bfloat16)
    return lax.dot_general(q, k, (((1,), (1,)), ((), ())),
                           preferred_element_type=jnp.float32)


def _exp_shifted(s):
    return jnp.exp2(s - jnp.max(s, axis=-1, keepdims=True))


def _inv_rowsum(p):
    return pl.reciprocal(jnp.sum(p, axis=-1, keepdims=True), approx=True)


@jax.jit
def pallas_standalone__mha_softmax__near_ridge_kernel(
    q: jax.Array,
    k: jax.Array,
    v: jax.Array,
):
    B, H, S, D = q.shape
    NH = B * H
    G, R = _GROUPS, _CARRY
    c = (D ** -0.5) * math.log2(math.e)
    tiles = range(S // _LANES)

    sizes = [n for n, cnt in _RUNS for _ in range(cnt)]
    starts = [sum(sizes[:i]) for i in range(len(sizes))]
    nb = len(sizes)
    assert sum(sizes) == NH - 1

    def segments(s0, n):
        out = []
        while n > 0:
            m = min(n, G - s0 % G)
            out.append((s0, m))
            s0, n = s0 + m, n - m
        return out

    after = {}
    for a, first, n in _WRITES:
        assert a >= first + n - 1
        ws = []
        for s0, m in segments(first, n):
            rows = _PIECE if m > 1 else S
            ws += [(s0, m, r0, rows) for r0 in range(0, S, rows)]
        for ci in range(0, len(ws), _MAX_STARTS):
            after[a + ci // _MAX_STARTS] = ws[ci:ci + _MAX_STARTS]

    def kernel(q_hbm, k_hbm, v_hbm, o_hbm, buf, p_scr, l_scr, s_scr, rsem, wsem):

        def start_read(a, s0, n, sem):
            hbm, shift = ((q_hbm, 0), (k_hbm, 0), (v_hbm, 1))[a]
            for s, m in segments(s0, n):
                pltpu.make_async_copy(
                    hbm.at[pl.ds(s % G, m), s // G],
                    buf.at[a, pl.ds(s + shift, m)], sem).start()

        def wait_filled(ref, sem):
            pltpu.make_async_copy(ref, ref, sem).wait()

        def start_writes(ws):
            for s, m, r0, rows in ws:
                pltpu.make_async_copy(
                    buf.at[_Q, pl.ds(s, m), pl.ds(r0, rows)],
                    o_hbm.at[pl.ds(s % G, m), s // G, pl.ds(r0, rows)],
                    wsem.at[0]).start()

        def begin_head(qh, kh):
            s = _scores(qh, kh, c)
            p = _exp_shifted(s[:R])
            cols = [p[:, t * _LANES:(t + 1) * _LANES] for t in tiles]
            l_scr[...] = (cols[0] + cols[1]) + (cols[2] + cols[3])
            for t in tiles:
                p_scr[t] = cols[t].astype(jnp.bfloat16)
            s_scr[...] = s[R:]

        def finish_head(vh):
            p = _exp_shifted(s_scr[...])
            p_all = jnp.concatenate(
                [jnp.concatenate([p_scr[t] for t in tiles], 1),
                 p.astype(jnp.bfloat16)], 0)
            o = jnp.dot(p_all, vh, preferred_element_type=jnp.float32)
            return jnp.concatenate(
                [o[:R] * _inv_rowsum(l_scr[...]), o[R:] * _inv_rowsum(p)],
                0).astype(jnp.bfloat16)

        def block(t, start2, *, b0, n, cnt):
            i = b0 + t
            start = starts[b0] + t * n
            wait_filled(buf.at[:, pl.ds(start + 1, n)], rsem.at[i])

            def load_q(h):
                if h < 2:
                    return buf[_Q, start + h]
                return jnp.concatenate(
                    [buf[_Q, start + h, pl.ds(0, _SPLIT), :],
                     buf[_Q, start2 + h, pl.ds(_SPLIT, S - _SPLIT), :]], 0)

            qs = {1: load_q(1)}
            for h in range(n):
                vh = buf[_V, start + h + 1]
                if h == 0:
                    buf[_Q, start] = finish_head(vh)
                else:
                    p = _exp_shifted(_scores(qs.pop(h), buf[_K, start + h], c))
                    o = jnp.dot(p.astype(jnp.bfloat16), vh,
                                preferred_element_type=jnp.float32)
                    buf[_Q, start + h] = (o * _inv_rowsum(p)).astype(jnp.bfloat16)
                for it in range(b0, b0 + cnt):
                    ws = after.get(starts[it] + h)
                    if ws:
                        pl.when(i == it)(functools.partial(start_writes, ws))
                if h + 2 <= n:
                    qs[h + 2] = load_q(h + 2)
            begin_head(qs.pop(n), buf[_K, start + n])
            return start2 + n

        def everything(done):
            start_read(_K, 0, 1, rsem.at[nb])
            start_read(_Q, 0, 1, rsem.at[nb])
            for i in range(nb):
                start_read(_V, starts[i], sizes[i], rsem.at[i])
                start_read(_K, starts[i] + 1, sizes[i], rsem.at[i])
                start_read(_Q, starts[i] + 1, sizes[i], rsem.at[i])
            start_read(_V, NH - 1, 1, rsem.at[nb + 1])

            wait_filled(buf.at[pl.ds(0, 2), pl.ds(0, 1)], rsem.at[nb])
            begin_head(buf[_Q, 0], buf[_K, 0])
            b0 = 0
            for n, cnt in _RUNS:
                done = lax.fori_loop(
                    0, cnt, functools.partial(block, b0=b0, n=n, cnt=cnt), done)
                b0 += cnt
            wait_filled(buf.at[_V, pl.ds(NH, 1)], rsem.at[nb + 1])
            o = finish_head(buf[_V, NH])
            cuts = (0,) + _TAIL_CUTS + (S,)
            for lo, hi in zip(cuts[:-1], cuts[1:]):
                buf[_Q, NH - 1, pl.ds(lo, hi - lo), :] = o[lo:hi]
                start_writes([(NH - 1, 1, lo, hi - lo)])
            wait_filled(o_hbm, wsem.at[0])
            return done + 1

        lax.while_loop(lambda done: done < NH, everything, jnp.int32(0))

    shp = (G, NH // G, S, D)
    spec = pl.BlockSpec(memory_space=pl.ANY)
    out = pl.pallas_call(
        kernel,
        in_specs=[spec] * 3,
        out_specs=spec,
        out_shape=jax.ShapeDtypeStruct(shp, q.dtype),
        scratch_shapes=[
            pltpu.VMEM((3, NH + 1, S, D), q.dtype),
            pltpu.VMEM((S // _LANES, R, _LANES), jnp.bfloat16),
            pltpu.VMEM((R, _LANES), jnp.float32),
            pltpu.VMEM((S - R, S), jnp.float32),
            pltpu.SemaphoreType.DMA((nb + 2,)),
            pltpu.SemaphoreType.DMA((1,)),
        ],
        compiler_params=pltpu.CompilerParams(
            vmem_limit_bytes=126 * 1024 * 1024,
            disable_bounds_checks=True,
            disable_semaphore_checks=True),
    )(q.reshape(shp), k.reshape(shp), v.reshape(shp))
    return out.reshape(B, H, S, D)
```

```python
import functools
import math

import jax
import jax.numpy as jnp
from jax import lax
import jax.experimental.pallas as pl
import jax.experimental.pallas.tpu as pltpu

_RUNS = ((1, 2), (2, 3), (4, 2), (7, 4), (17, 3), (32, 5))
_WRITES = ((187, 0, 184), (231, 184, 48), (247, 232, 16), (251, 248, 4),
           (253, 252, 2), (254, 254, 1))
_GROUPS = 32
_PIECE = 128
_MAX_STARTS = 16
_SPLIT = 448
_CARRY = 256
_TAIL_CUTS = (128, 256, 384, 464)
_LANES = 128
_Q, _K, _V = 0, 1, 2


def _scores(q, k):
    return lax.dot_general(q, k, (((1,), (1,)), ((), ())),
                           preferred_element_type=jnp.float32)


def _exp_shifted(s, c):
    return jnp.exp2((s - jnp.max(s, axis=-1, keepdims=True)) * c)


def _inv_rowsum(p):
    return pl.reciprocal(jnp.sum(p, axis=-1, keepdims=True), approx=True)


@jax.jit
def pallas_standalone__mha_softmax__near_ridge_kernel(
    q: jax.Array,
    k: jax.Array,
    v: jax.Array,
):
    B, H, S, D = q.shape
    NH = B * H
    G, R = _GROUPS, _CARRY
    c = (D ** -0.5) * math.log2(math.e)
    tiles = range(S // _LANES)

    sizes = [n for n, cnt in _RUNS for _ in range(cnt)]
    starts = [sum(sizes[:i]) for i in range(len(sizes))]
    nb = len(sizes)
    assert sum(sizes) == NH - 1

    def segments(s0, n):
        out = []
        while n > 0:
            m = min(n, G - s0 % G)
            out.append((s0, m))
            s0, n = s0 + m, n - m
        return out

    after = {}
    for a, first, n in _WRITES:
        assert a >= first + n - 1
        ws = []
        for s0, m in segments(first, n):
            rows = _PIECE if m > 1 else S
            ws += [(s0, m, r0, rows) for r0 in range(0, S, rows)]
        for ci in range(0, len(ws), _MAX_STARTS):
            after[a + ci // _MAX_STARTS] = ws[ci:ci + _MAX_STARTS]

    def kernel(q_hbm, k_hbm, v_hbm, o_hbm, buf, p_scr, l_scr, s_scr, rsem, wsem):

        def start_read(a, s0, n, sem):
            hbm, shift = ((q_hbm, 0), (k_hbm, 0), (v_hbm, 1))[a]
            for s, m in segments(s0, n):
                pltpu.make_async_copy(
                    hbm.at[pl.ds(s % G, m), s // G],
                    buf.at[a, pl.ds(s + shift, m)], sem).start()

        def wait_filled(ref, sem):
            pltpu.make_async_copy(ref, ref, sem).wait()

        def start_writes(ws):
            for s, m, r0, rows in ws:
                pltpu.make_async_copy(
                    buf.at[_Q, pl.ds(s, m), pl.ds(r0, rows)],
                    o_hbm.at[pl.ds(s % G, m), s // G, pl.ds(r0, rows)],
                    wsem.at[0]).start()

        def begin_head(qh, kh):
            s = _scores(qh, kh)
            p = _exp_shifted(s[:R], c)
            cols = [p[:, t * _LANES:(t + 1) * _LANES] for t in tiles]
            l_scr[...] = (cols[0] + cols[1]) + (cols[2] + cols[3])
            for t in tiles:
                p_scr[t] = cols[t].astype(jnp.bfloat16)
            s_scr[...] = s[R:]

        def finish_head(vh):
            p = _exp_shifted(s_scr[...], c)
            p_all = jnp.concatenate(
                [jnp.concatenate([p_scr[t] for t in tiles], 1),
                 p.astype(jnp.bfloat16)], 0)
            o = jnp.dot(p_all, vh, preferred_element_type=jnp.float32)
            return jnp.concatenate(
                [o[:R] * _inv_rowsum(l_scr[...]), o[R:] * _inv_rowsum(p)],
                0).astype(jnp.bfloat16)

        def block(t, start2, *, b0, n, cnt):
            i = b0 + t
            start = starts[b0] + t * n
            wait_filled(buf.at[:, pl.ds(start + 1, n)], rsem.at[i])

            def load_q(h):
                if h < 2:
                    return buf[_Q, start + h]
                return jnp.concatenate(
                    [buf[_Q, start + h, pl.ds(0, _SPLIT), :],
                     buf[_Q, start2 + h, pl.ds(_SPLIT, S - _SPLIT), :]], 0)

            qs = {1: load_q(1)}
            for h in range(n):
                vh = buf[_V, start + h + 1]
                if h == 0:
                    buf[_Q, start] = finish_head(vh)
                else:
                    p = _exp_shifted(_scores(qs.pop(h), buf[_K, start + h]), c)
                    o = jnp.dot(p.astype(jnp.bfloat16), vh,
                                preferred_element_type=jnp.float32)
                    buf[_Q, start + h] = (o * _inv_rowsum(p)).astype(jnp.bfloat16)
                for it in range(b0, b0 + cnt):
                    ws = after.get(starts[it] + h)
                    if ws:
                        pl.when(i == it)(functools.partial(start_writes, ws))
                if h + 2 <= n:
                    qs[h + 2] = load_q(h + 2)
            begin_head(qs.pop(n), buf[_K, start + n])
            return start2 + n

        def everything(done):
            start_read(_K, 0, 1, rsem.at[nb])
            start_read(_Q, 0, 1, rsem.at[nb])
            for i in range(nb):
                start_read(_V, starts[i], sizes[i], rsem.at[i])
                start_read(_K, starts[i] + 1, sizes[i], rsem.at[i])
                start_read(_Q, starts[i] + 1, sizes[i], rsem.at[i])
            start_read(_V, NH - 1, 1, rsem.at[nb + 1])

            wait_filled(buf.at[pl.ds(0, 2), pl.ds(0, 1)], rsem.at[nb])
            begin_head(buf[_Q, 0], buf[_K, 0])
            b0 = 0
            for n, cnt in _RUNS:
                done = lax.fori_loop(
                    0, cnt, functools.partial(block, b0=b0, n=n, cnt=cnt), done)
                b0 += cnt
            wait_filled(buf.at[_V, pl.ds(NH, 1)], rsem.at[nb + 1])
            o = finish_head(buf[_V, NH])
            cuts = (0,) + _TAIL_CUTS + (S,)
            for lo, hi in zip(cuts[:-1], cuts[1:]):
                buf[_Q, NH - 1, pl.ds(lo, hi - lo), :] = o[lo:hi]
                start_writes([(NH - 1, 1, lo, hi - lo)])
            wait_filled(o_hbm, wsem.at[0])
            return done + 1

        lax.while_loop(lambda done: done < NH, everything, jnp.int32(0))

    shp = (G, NH // G, S, D)
    spec = pl.BlockSpec(memory_space=pl.ANY)
    out = pl.pallas_call(
        kernel,
        in_specs=[spec] * 3,
        out_specs=spec,
        out_shape=jax.ShapeDtypeStruct(shp, q.dtype),
        scratch_shapes=[
            pltpu.VMEM((3, NH + 1, S, D), q.dtype),
            pltpu.VMEM((S // _LANES, R, _LANES), jnp.bfloat16),
            pltpu.VMEM((R, _LANES), jnp.float32),
            pltpu.VMEM((S - R, S), jnp.float32),
            pltpu.SemaphoreType.DMA((nb + 2,)),
            pltpu.SemaphoreType.DMA((1,)),
        ],
        compiler_params=pltpu.CompilerParams(
            vmem_limit_bytes=112 * 1024 * 1024,
            disable_bounds_checks=True,
            disable_semaphore_checks=True),
    )(q.reshape(shp), k.reshape(shp), v.reshape(shp))
    return out.reshape(B, H, S, D)
```
